```python
import jax
import jax.numpy as jnp

def _softmax(x, axis=-1):
    return jax.nn.softmax(x, axis=axis)
def _gelu(x):
    return jax.nn.gelu(x, approximate=True)
def _silu(x):
    return jax.nn.silu(x)
def _sigmoid(x):
    return jax.nn.sigmoid(x)
def _layernorm(x, axis=-1, eps=1e-5):
    m = jnp.mean(x, axis=axis, keepdims=True)
    v = jnp.var(x, axis=axis, keepdims=True)
    return (x - m) / jnp.sqrt(v + eps)
def _scatter_add(tgt, idx, src, axis=0):
    return tgt.at[idx].add(src)
def _segment_sum(src, seg, n):
    return jax.ops.segment_sum(src, seg, n)
class _Rng:
    def __init__(self, key):
        self._k = key
    def _next(self):
        self._k, sub = jax.random.split(self._k)
        return sub
    def normal(self, shape):
        return jax.random.normal(self._next(), shape, dtype=jnp.bfloat16)
    def randint(self, lo, hi, shape):
        return jax.random.randint(self._next(), shape, lo, hi, dtype=jnp.int32)
    def uniform(self, shape, lo=0.0, hi=1.0):
        return jax.random.uniform(self._next(), shape, jnp.bfloat16, lo, hi)
    def permutation(self, n):
        return jax.random.permutation(self._next(), n)


kernel_name = 'concat_heads__gqa_block_cached__mha_block_cached__near_ridge'

def setup_inputs():
    _rng = _Rng(jax.random.key(int.from_bytes(__import__("os").urandom(4), "little")))
    _w = (lambda a: (lambda t: t.astype(jnp.bfloat16) if jnp.issubdtype(t.dtype, jnp.floating) else t)(jnp.asarray(a)))
    def _A_setup():
        B, Sq, D = 16, 160, 640
        Hq, Hkv, Sk, Dh = 32, 32, 512, 192
        assert Hq % Hkv == 0, (Hq, Hkv)
        return {
            "x": _w((lambda *s: _rng.normal(s) * 0.05)(B, Sq, D)),
            "k_cache": _w((lambda *s: _rng.normal(s) * 0.05)(B, Hkv, Sk, Dh)),
            "v_cache": _w((lambda *s: _rng.normal(s) * 0.05)(B, Hkv, Sk, Dh)),
            "wq": _w((lambda *s: _rng.normal(s) * 0.05)(D, Hq * Dh) * (D ** -0.5)),
            "wo": _w((lambda *s: _rng.normal(s) * 0.05)(Hq * Dh, D) * ((Hq * Dh) ** -0.5)),
        }
    _A_in = _A_setup()

    def _B_setup():
        B, Sq, D = 16, 160, 640
        H, Sk, Dh = 32, 512, 192
        return {
            "x": _w((lambda *s: _rng.normal(s) * 0.05)(B, Sq, D)),
            "k_cache": _w((lambda *s: _rng.normal(s) * 0.05)(B, H, Sk, Dh)),
            "v_cache": _w((lambda *s: _rng.normal(s) * 0.05)(B, H, Sk, Dh)),
            "wq": _w((lambda *s: _rng.normal(s) * 0.05)(D, H * Dh) * (D ** -0.5)),
            "wo": _w((lambda *s: _rng.normal(s) * 0.05)(H * Dh, D) * ((H * Dh) ** -0.5)),
        }
    _B_in = _B_setup()

    return {
        "A_x": _A_in["x"],
        "A_k_cache": _A_in["k_cache"],
        "A_v_cache": _A_in["v_cache"],
        "A_wq": _A_in["wq"],
        "A_wo": _A_in["wo"],
        "B_x": _B_in["x"],
        "B_k_cache": _B_in["k_cache"],
        "B_v_cache": _B_in["v_cache"],
        "B_wq": _B_in["wq"],
        "B_wo": _B_in["wo"],
    }

def reference(A_x, A_k_cache, A_v_cache, A_wq, A_wo, B_x, B_k_cache, B_v_cache, B_wq, B_wo):
    def _A_ref(x, k_cache, v_cache, wq, wo):
        B, Sq, D = x.shape
        Hq, Dh = 32, 192
        Hkv = k_cache.shape[1]
        rep = Hq // Hkv
        q = (lambda x, *d: x.transpose(*d))((x @ wq).reshape(B, Sq, Hq, Dh), 0, 2, 1, 3)
        k = jnp.repeat(k_cache, rep, axis=1)
        v = jnp.repeat(v_cache, rep, axis=1)
        scores = jnp.einsum("bhqd,bhkd->bhqk", q, k) * (Dh ** -0.5)
        p = _softmax(scores, axis=-1)
        o = jnp.einsum("bhqk,bhkd->bhqd", p, v)
        return (lambda x, *d: x.transpose(*d))(o, 0, 2, 1, 3).reshape(B, Sq, Hq * Dh) @ wo

    def _B_ref(x, k_cache, v_cache, wq, wo):
        B, Sq, D = x.shape
        H, Dh = 32, 192
        q = (lambda x, *d: x.transpose(*d))((x @ wq).reshape(B, Sq, H, Dh), 0, 2, 1, 3)
        scores = jnp.einsum("bhqd,bhkd->bhqk", q, k_cache) * (Dh ** -0.5)
        p = _softmax(scores, axis=-1)
        o = jnp.einsum("bhqk,bhkd->bhqd", p, v_cache)
        return (lambda x, *d: x.transpose(*d))(o, 0, 2, 1, 3).reshape(B, Sq, H * Dh) @ wo

    a = _A_ref(A_x, A_k_cache, A_v_cache, A_wq, A_wo)
    b = _B_ref(B_x, B_k_cache, B_v_cache, B_wq, B_wo)
    return jnp.concatenate([a, b], axis=-1)
```

```python
import jax
import jax.numpy as jnp
import numpy as np
from jax import lax
import jax.experimental.pallas as pl
import jax.experimental.pallas.tpu as pltpu

B, SQ, D = 16, 160, 640
H, SK, DH = 32, 512, 192
PW = 2 * DH
NP = H // 2
QSCALE = float(DH ** -0.5 * np.log2(np.e))

NN = (((1,), (0,)), ((), ()))
NT = (((1,), (1,)), ((), ()))
f32, bf16 = jnp.float32, jnp.bfloat16


def make(nb=2, vmem_mb=100, flags=None):
    M = nb * SQ
    NBC = B // nb

    def kernel(ax, ak, av, awq, awo, bx, bk, bv, bwq, bwo, out_ref, acc_a, acc_b):
        g = pl.program_id(0)
        c = pl.program_id(1)
        rows = pl.ds(pl.multiple_of(c * M, M), M)

        @pl.when(g == 0)
        def _():
            acc_a[rows, :] = jnp.zeros((M, D), jnp.float32)
            acc_b[rows, :] = jnp.zeros((M, D), jnp.float32)

        br = ((ax, ak, av, awq, awo, acc_a), (bx, bk, bv, bwq, bwo, acc_b))
        units = [(r, i) for r in range(2) for i in range(nb)]
        lane = lax.broadcasted_iota(jnp.int32, (SQ, 128), 1)
        lo = lane < 64

        def urows(u):
            return pl.ds(pl.multiple_of(c * M + u[1] * SQ, SQ), SQ)

        def Q(u):
            x_ref, _, _, wq_ref, _, _ = br[u[0]]
            q = lax.dot_general(x_ref[urows(u), :], wq_ref[...], NN, preferred_element_type=f32) * QSCALE
            q0, q1, q2 = q[:, 0:128], q[:, 128:256], q[:, 256:384]
            qa = jnp.concatenate([q0, jnp.where(lo, q1, 0.0)], axis=1).astype(bf16)
            qb = jnp.concatenate([jnp.where(lo, 0.0, q1), q2], axis=1).astype(bf16)
            return qa, qb

        def S(u, qq, r0):
            k_ref = br[u[0]][1]
            s = lax.dot_general(qq, k_ref[u[1], r0:r0 + 256, :], NN, preferred_element_type=f32)
            m = jnp.max(s, axis=-1, keepdims=True)
            p = jnp.exp2(s - m)
            l = jnp.sum(p, axis=-1, keepdims=True)
            r = pl.reciprocal(l, approx=True)
            r = r * (2.0 - l * r)
            return p.astype(bf16), r

        def PV(u, pr, r0):
            v_ref = br[u[0]][2]
            p, r = pr
            return lax.dot_general(p, v_ref[u[1], r0:r0 + 256, :], NT, preferred_element_type=f32) * r

        def O(u, oa, ob):
            wo_ref, acc = br[u[0]][4:6]
            o = jnp.concatenate([oa[:, 0:128], jnp.where(lo, oa[:, 128:256], ob[:, 0:128]), ob[:, 128:256]], axis=1).astype(bf16)
            acc[urows(u), :] += lax.dot_general(o, wo_ref[...], NN, preferred_element_type=f32)

        n = len(units)
        q = {0: Q(units[0])}
        if n > 1:
            q[1] = Q(units[1])
        o = {}
        for j, u in enumerate(units):
            pa = S(u, q[j][0], 0)
            pb = S(u, q[j][1], 128)
            if j >= 1:
                O(units[j - 1], *o[j - 1])
            if j + 2 < n:
                q[j + 2] = Q(units[j + 2])
            o[j] = (PV(u, pa, 0), PV(u, pb, 128))
        O(units[n - 1], *o[n - 1])

        @pl.when(g == NP - 1)
        def _():
            out_ref[:, 0:D] = acc_a[rows, :].astype(out_ref.dtype)
            out_ref[:, D:2 * D] = acc_b[rows, :].astype(out_ref.dtype)

    x_spec = pl.BlockSpec((B * SQ, D), lambda g, c: (0, 0), pipeline_mode=pl.Buffered(1))
    kv_spec = pl.BlockSpec((nb, PW, SK), lambda g, c: (c, g, 0))
    wq_spec = pl.BlockSpec((D, PW), lambda g, c: (0, g))
    wo_spec = pl.BlockSpec((PW, D), lambda g, c: (g, 0))
    out_spec = pl.BlockSpec((M, 2 * D), lambda g, c: (jnp.where(g == NP - 1, c, 0), 0))

    @jax.jit
    def fn(A_x, A_k_cache, A_v_cache, A_wq, A_wo, B_x, B_k_cache, B_v_cache, B_wq, B_wo):
        t = lambda a: jnp.swapaxes(a, 2, 3).reshape(B, H * DH, SK)
        f = lambda a: a.reshape(B * SQ, D)
        out = pl.pallas_call(
            kernel,
            grid=(NP, NBC),
            in_specs=[x_spec, kv_spec, kv_spec, wq_spec, wo_spec] * 2,
            out_specs=out_spec,
            out_shape=jax.ShapeDtypeStruct((B * SQ, 2 * D), A_x.dtype),
            scratch_shapes=[pltpu.VMEM((B * SQ, D), jnp.float32)] * 2,
            compiler_params=pltpu.CompilerParams(
                dimension_semantics=("arbitrary", "arbitrary"),
                vmem_limit_bytes=vmem_mb * 1024 * 1024, flags=flags),
            name="attn",
        )(f(A_x), t(A_k_cache), t(A_v_cache), A_wq, A_wo, f(B_x), t(B_k_cache), t(B_v_cache), B_wq, B_wo)
        return out.reshape(B, SQ, 2 * D)
    return fn


_fn = make(nb=4)


@jax.jit
def pallas_concat_heads__gqa_block_cached__mha_block_cached__near_ridge_kernel(
    A_x, A_k_cache, A_v_cache, A_wq, A_wo, B_x, B_k_cache, B_v_cache, B_wq, B_wo
):
    return _fn(A_x, A_k_cache, A_v_cache, A_wq, A_wo, B_x, B_k_cache, B_v_cache, B_wq, B_wo)
```

```python
import jax
import jax.numpy as jnp
import numpy as np
from jax import lax
import jax.experimental.pallas as pl
import jax.experimental.pallas.tpu as pltpu

B, SQ, D = 16, 160, 640
H, SK, DH = 32, 512, 192
PW = 2 * DH
NP = H // 2
UG = 2 * B
NU = NP * UG
QM = 128
QL = SQ - QM
QSCALE = float(DH ** -0.5 * np.log2(np.e))

NN = (((1,), (0,)), ((), ()))
NT = (((1,), (1,)), ((), ()))
f32, bf16 = jnp.float32, jnp.bfloat16


def _nn(a, b):
    return lax.dot_general(a, b, NN, preferred_element_type=f32)


def _nt(a, b):
    return lax.dot_general(a, b, NT, preferred_element_type=f32)


def make(n=8, R=8, order='abmzt', seq='PABQO', vmem_mb=110, flags=None, XL=6, ramp=(99,), p0=99, pr=0):
    flags = dict(flags or {}, XLA_TPU_RESCHEDULE_DMA_DONES=True)
    T = NU // n
    TG = UG // n
    R = min(R, n)
    assert n % R == 0 and R % 2 == 0

    def kernel(ax, ak, av, awq, awo, bx, bk, bv, bwq, bwo, out_hbm,
               x_buf, wq_buf, wo_buf, k_buf, v_buf, acc, o_buf, q_c, p_c, r_c,
               sems, o_sem):
        x_hbm, k_hbm, v_hbm = (ax, bx), (ak, bk), (av, bv)
        wq_hbm, wo_hbm = (awq, bwq), (awo, bwo)
        lo = lax.broadcasted_iota(jnp.int32, (SQ, 128), 1) < 64
        lo_m = lax.broadcasted_iota(jnp.int32, (QM, 128), 1) < 64
        lo_l = lax.broadcasted_iota(jnp.int32, (QL, 128), 1) < 64

        def al(i, m):
            return i if isinstance(i, int) else pl.multiple_of(i, m)

        def gb(jh):
            return (jh >> 4) & (NP - 1), jh & (B - 1)

        def when(cond, f):
            if isinstance(cond, bool):
                if cond:
                    f()
            else:
                pl.when(cond)(f)

        def k_copy(r, jh, slot):
            g, b = gb(jh)
            return pltpu.make_async_copy(k_hbm[r].at[b, pl.ds(al(g * PW, PW), PW), :], k_buf.at[slot], sems.at[slot])

        def v_copy(r, jh, slot):
            g, b = gb(jh)
            return pltpu.make_async_copy(v_hbm[r].at[b, pl.ds(al(g * PW, PW), PW), :], v_buf.at[slot], sems.at[R + slot])

        def x_copy(r, jh):
            b = jh & (B - 1)
            return pltpu.make_async_copy(x_hbm[r].at[b], x_buf.at[r, b], sems.at[2 * R + 5 + r * B + b])

        def wq_copy(r, g):
            return pltpu.make_async_copy(wq_hbm[r].at[:, pl.ds(al(g * PW, 128), PW)], wq_buf.at[r, g], sems.at[2 * R + r])

        def wo_copy(r, g):
            return pltpu.make_async_copy(wo_hbm[r].at[pl.ds(al(g * PW, PW), PW), :], wo_buf.at[r, g], sems.at[2 * R + 2 + r])

        def out_copy(r, b):
            return pltpu.make_async_copy(o_buf.at[r, b], out_hbm.at[b, :, pl.ds(r * D, D)], o_sem)

        def Q(r, jh):
            g, b = gb(jh)
            q = _nn(x_buf[r, b], wq_buf[r, g]) * QSCALE
            q0, q1, q2 = q[:, 0:128], q[:, 128:256], q[:, 256:384]
            qa = jnp.concatenate([q0, jnp.where(lo, q1, 0.0)], axis=1).astype(bf16)
            qb = jnp.concatenate([jnp.where(lo, 0.0, q1), q2], axis=1).astype(bf16)
            return qa, qb

        def S(qq, slot, r0):
            s = _nn(qq, k_buf[slot, r0:r0 + 256, :])
            m = jnp.max(s, axis=-1, keepdims=True)
            p = jnp.exp2(s - m)
            l = jnp.sum(p, axis=-1, keepdims=True)
            rl = pl.reciprocal(l, approx=True)
            rl = rl * (2.0 - l * rl)
            return p.astype(bf16), jnp.broadcast_to(rl, (SQ, 128))

        def PV(slot, pa, ra, pb, rb):
            fs = dict(
                z=lambda: _nt(pa, v_buf[slot, 0:128, :]),
                t=lambda: _nt(pb, v_buf[slot, 256:384, :]),
                a=lambda: _nt(v_buf[slot, 128:192, :], pa[:QM]),
                b=lambda: _nt(v_buf[slot, 192:256, :], pb[:QM]),
                m=lambda: _nt(jnp.concatenate([pa[QM:], pb[QM:]], axis=0), v_buf[slot, 128:256, :]),
            )
            o = {k: fs[k]() for k in order}
            om = jnp.concatenate([o['a'], o['b']], axis=0).T * jnp.where(lo_m, ra[:QM], rb[:QM])
            ol = jnp.where(lo_l, o['m'][:QL] * ra[QM:], o['m'][QL:] * rb[QM:])
            return jnp.concatenate([o['z'] * ra, jnp.concatenate([om, ol], axis=0), o['t'] * rb], axis=1).astype(bf16)

        def O(r, jh, o):
            g, b = gb(jh)
            tot = jnp.where(g == 0, 0.0, acc[r, b]) + _nn(o, wo_buf[r, g])
            acc[r, b] = tot
            o_buf[r, b] = tot.astype(o_buf.dtype)

        first = [(-2, lambda: wq_copy(0, 0)), (-2, lambda: x_copy(0, 0))]
        for j in range(max(R, XL, 3)):
            if j < R:
                first.append((j, lambda j=j: k_copy(j % 2, j // 2, j)))
            if 1 <= j < R:
                first.append((j, lambda j=j: v_copy((j - 1) % 2, (j - 1) // 2, j - 1)))
            if j == 0:
                first.append((j, lambda: wq_copy(1, 0)))
            if j < XL:
                first.append((j, lambda j=j: x_copy((j + 1) % 2, (j + 1) // 2)))
            if j in (1, 2):
                first.append((j, lambda j=j: wo_copy(j - 1, 0)))
        ends = np.minimum(np.cumsum((0,) + tuple(ramp)), len(first))
        assert ends[-1] == len(first)

        def issue(point):
            if point + 3 < len(ends):
                for i in range(ends[point + 2], ends[point + 3]):
                    need, f = first[i]
                    assert need >= point
                    f().start(priority=0 if i < p0 else 1)

        issue(-2)
        wq_copy(0, 0).wait()
        x_copy(0, 0).wait()
        issue(-1)
        q_c[0], q_c[1] = Q(0, 0)

        def body(t, carry):
            g = t // TG if TG == 1 else t >> (TG.bit_length() - 1)
            c = t & (TG - 1)
            jh0 = t * (n // 2)

            def at(ju, pos):
                if ju % n != pos:
                    return False
                return True if TG == 1 else c == ju // n

            def both(a, b):
                if a is False or b is False:
                    return False
                if a is True:
                    return b
                return jnp.logical_and(a, b)

            more = g < NP - 1
            gn = jnp.minimum(g + 1, NP - 1)
            q = (q_c[0], q_c[1])
            p = (p_c[0], r_c[0], p_c[1], r_c[1])
            for pos in range(n):
                j = t * n + pos
                r, jh = pos % 2, jh0 + pos // 2
                ro = (pos + 1) % 2
                jhp, jhn = jh0 + (pos - 1) // 2, jh0 + (pos + 1) // 2
                sk, sv = pos % R, (pos - 1) % R
                if pos + 3 < len(ends):
                    when(t == 0, lambda: issue(pos))
                for st in seq:
                    if st == 'P':
                        when(True if pos else t > 0, lambda: v_copy(ro, jhp, sv).wait())
                        o = PV(sv, *p)
                        when(True if pos - 1 + R < n else t < T - 1, lambda: v_copy(ro, jhp + R // 2, sv).start(priority=pr))
                    elif st == 'A':
                        k_copy(r, jh, sk).wait()
                        pna = S(q[0], sk, 0)
                    elif st == 'B':
                        pn = pna + S(q[1], sk, 128)
                        when(True if pos + R < n else t < T - 1, lambda: k_copy(r, jh + R // 2, sk).start(priority=pr))
                    elif st == 'Q':
                        when(both(at(UG - 1, pos), more), lambda: wq_copy(0, gn).wait())
                        when(at(0, pos), lambda: wq_copy(1, g).wait())
                        when(j + 1 < UG, lambda: x_copy(ro, jhn).wait())
                        qn = Q(ro, jhn)
                        when(j + 1 + XL < UG, lambda: x_copy((pos + 1 + XL) % 2, jh0 + (pos + 1 + XL) // 2).start(priority=pr))
                    elif st == 'O':
                        when(at(1, pos), lambda: wo_copy(0, g).wait())
                        when(at(2, pos), lambda: wo_copy(1, g).wait())
                        O(ro, jhp, o)
                        when(jhp >= (NP - 1) * B, lambda: out_copy(ro, jhp & (B - 1)).start())
                when(both(at(10, pos), more), lambda: wq_copy(0, gn).start(priority=pr))
                when(both(at(14, pos), more), lambda: wq_copy(1, gn).start(priority=pr))
                when(both(at(18, pos), more), lambda: wo_copy(0, gn).start(priority=pr))
                when(both(at(22, pos), more), lambda: wo_copy(1, gn).start(priority=pr))
                q, p = qn, pn
            q_c[0], q_c[1] = q
            p_c[0], r_c[0], p_c[1], r_c[1] = p
            return carry

        lax.fori_loop(0, T, body, 0)

        jl = NU // 2 - 1
        v_copy(1, jl, R - 1).wait()
        O(1, jl, PV(R - 1, p_c[0], r_c[0], p_c[1], r_c[1]))
        out_copy(1, B - 1).start()
        pltpu.make_async_copy(o_buf, o_buf, o_sem).wait()

    @jax.jit
    def fn(A_x, A_k_cache, A_v_cache, A_wq, A_wo, B_x, B_k_cache, B_v_cache, B_wq, B_wo):
        tr = lambda a: jnp.swapaxes(a, 2, 3).reshape(B, H * DH, SK)
        return pl.pallas_call(
            kernel,
            in_specs=[pl.BlockSpec(memory_space=pl.ANY)] * 10,
            out_specs=pl.BlockSpec(memory_space=pl.ANY),
            out_shape=jax.ShapeDtypeStruct((B, SQ, 2 * D), A_x.dtype),
            scratch_shapes=[
                pltpu.VMEM((2, B, SQ, D), bf16),
                pltpu.VMEM((2, NP, D, PW), bf16),
                pltpu.VMEM((2, NP, PW, D), bf16),
                pltpu.VMEM((R, PW, SK), bf16),
                pltpu.VMEM((R, PW, SK), bf16),
                pltpu.VMEM((2, B, SQ, D), f32),
                pltpu.VMEM((2, B, SQ, D), A_x.dtype),
                pltpu.VMEM((2, SQ, 256), bf16),
                pltpu.VMEM((2, SQ, SK), bf16),
                pltpu.VMEM((2, SQ, 128), f32),
                pltpu.SemaphoreType.DMA((2 * R + 5 + 2 * B,)),
                pltpu.SemaphoreType.DMA,
            ],
            compiler_params=pltpu.CompilerParams(vmem_limit_bytes=vmem_mb * 1024 * 1024, flags=flags, disable_bounds_checks=True),
            name="attn",
        )(A_x, tr(A_k_cache), tr(A_v_cache), A_wq, A_wo, B_x, tr(B_k_cache), tr(B_v_cache), B_wq, B_wo)
    return fn


_fn = make(n=16, seq='PAQBO')


@jax.jit
def pallas_concat_heads__gqa_block_cached__mha_block_cached__near_ridge_kernel(
    A_x, A_k_cache, A_v_cache, A_wq, A_wo, B_x, B_k_cache, B_v_cache, B_wq, B_wo
):
    return _fn(A_x, A_k_cache, A_v_cache, A_wq, A_wo, B_x, B_k_cache, B_v_cache, B_wq, B_wo)
```

```python
import jax
import jax.numpy as jnp
import numpy as np
from jax import lax
import jax.experimental.pallas as pl
import jax.experimental.pallas.tpu as pltpu

B, SQ, D = 16, 160, 640
H, SK, DH = 32, 512, 192
PW = 2 * DH
NP = H // 2
UG = 2 * B
NU = NP * UG
QM = 128
QL = SQ - QM
QSCALE = float(DH ** -0.5 * np.log2(np.e))

NN = (((1,), (0,)), ((), ()))
NT = (((1,), (1,)), ((), ()))
f32, bf16 = jnp.float32, jnp.bfloat16


def _nn(a, b):
    return lax.dot_general(a, b, NN, preferred_element_type=f32)


def _nt(a, b):
    return lax.dot_general(a, b, NT, preferred_element_type=f32)


def make(n=8, R=8, seq='ABztabmQO', vmem_mb=110, flags=None, XL=6, DL=2):
    flags = dict(flags or {}, XLA_TPU_RESCHEDULE_DMA_DONES=True)
    T = NU // n
    TG = UG // n
    R = min(R, n)
    assert n % R == 0 and R % 2 == 0

    def kernel(ax, ak, av, awq, awo, bx, bk, bv, bwq, bwo, out_hbm,
               x_buf, wq_buf, wo_buf, k_buf, v_buf, acc, o_buf, q_c, sems, o_sem):
        x_hbm, k_hbm, v_hbm = (ax, bx), (ak, bk), (av, bv)
        wq_hbm, wo_hbm = (awq, bwq), (awo, bwo)
        lo = lax.broadcasted_iota(jnp.int32, (SQ, 128), 1) < 64
        lo_m = lax.broadcasted_iota(jnp.int32, (QM, 128), 1) < 64
        lo_l = lax.broadcasted_iota(jnp.int32, (QL, 128), 1) < 64

        def al(i, m):
            return i if isinstance(i, int) else pl.multiple_of(i, m)

        def gb(jh):
            return (jh >> 4) & (NP - 1), jh & (B - 1)

        def when(cond, f):
            if isinstance(cond, bool):
                if cond:
                    f()
            else:
                pl.when(cond)(f)

        def k_copy(jh0, d):
            g, b = gb(jh0 + d // 2)
            return pltpu.make_async_copy(k_hbm[d % 2].at[b, pl.ds(al(g * PW, PW), PW), :], k_buf.at[d % R], sems.at[d % R])

        def v_copy(jh0, d):
            g, b = gb(jh0 + d // 2)
            return pltpu.make_async_copy(v_hbm[d % 2].at[b, pl.ds(al(g * PW, PW), PW), :], v_buf.at[d % R], sems.at[R + d % R])

        def x_copy(jh0, d):
            r, b = d % 2, (jh0 + d // 2) & (B - 1)
            return pltpu.make_async_copy(x_hbm[r].at[b], x_buf.at[r, b], sems.at[2 * R + 4 + r * B + b])

        def wq_copy(r, g):
            return pltpu.make_async_copy(wq_hbm[r].at[:, pl.ds(al(g * PW, 128), PW)], wq_buf.at[r, g], sems.at[2 * R + r])

        def wo_copy(r, g):
            return pltpu.make_async_copy(wo_hbm[r].at[pl.ds(al(g * PW, PW), PW), :], wo_buf.at[r, g], sems.at[2 * R + 2 + r])

        def out_copy(r, b):
            return pltpu.make_async_copy(o_buf.at[r, b], out_hbm.at[b, :, pl.ds(r * D, D)], o_sem)

        def Q(r, jh):
            g, b = gb(jh)
            q = _nn(x_buf[r, b], wq_buf[r, g]) * QSCALE
            q0, q1, q2 = q[:, 0:128], q[:, 128:256], q[:, 256:384]
            qa = jnp.concatenate([q0, jnp.where(lo, q1, 0.0)], axis=1).astype(bf16)
            qb = jnp.concatenate([jnp.where(lo, 0.0, q1), q2], axis=1).astype(bf16)
            return qa, qb

        def softmax(s):
            m = jnp.max(s, axis=-1, keepdims=True)
            p = jnp.exp2(s - m)
            l = jnp.sum(p, axis=-1, keepdims=True)
            rl = pl.reciprocal(l, approx=True)
            rl = rl * (2.0 - l * rl)
            return (p.astype(bf16), p[:QM].astype(bf16), p[QM:].astype(bf16)), jnp.broadcast_to(rl, (SQ, 128))

        def pv_part(k, slot, pa, pb):
            if k == 'z':
                return _nt(pa[0], v_buf[slot, 0:128, :])
            if k == 't':
                return _nt(pb[0], v_buf[slot, 256:384, :])
            if k == 'a':
                return _nt(v_buf[slot, 128:192, :], pa[1])
            if k == 'b':
                return _nt(v_buf[slot, 192:256, :], pb[1])
            return _nt(jnp.concatenate([pa[2], pb[2]], axis=0), v_buf[slot, 128:256, :])

        def pv_join(o, ra, rb):
            om = jnp.concatenate([o['a'], o['b']], axis=0).T * jnp.where(lo_m, ra[:QM], rb[:QM])
            ol = jnp.where(lo_l, o['m'][:QL] * ra[QM:], o['m'][QL:] * rb[QM:])
            return jnp.concatenate([o['z'] * ra, jnp.concatenate([om, ol], axis=0), o['t'] * rb], axis=1).astype(bf16)

        def O(r, jh, o):
            g, b = gb(jh)
            tot = jnp.where(g == 0, 0.0, acc[r, b]) + _nn(o, wo_buf[r, g])
            acc[r, b] = tot
            o_buf[r, b] = tot.astype(o_buf.dtype)

        wq_copy(0, 0).start()
        x_copy(0, 0).start()
        lead = ''.join(c for c in seq if c in 'AQOabmzt')
        for j in range(max(R, XL, 3)):
            seen = set()
            for c in lead:
                c = 'P' if c.islower() else c
                if c in seen:
                    continue
                seen.add(c)
                if c == 'A' and j < R - DL:
                    k_copy(0, j).start()
                if c == 'P' and j < R - DL:
                    v_copy(0, j).start()
                if c == 'Q' and j == 0:
                    wq_copy(1, 0).start()
                if c == 'Q' and j < XL:
                    x_copy(0, j + 1).start()
                if c == 'O' and j in (0, 1):
                    wo_copy(j, 0).start()
        wq_copy(0, 0).wait()
        x_copy(0, 0).wait()
        q_c[0], q_c[1] = Q(0, 0)

        def body(t, carry):
            g = t >> (TG.bit_length() - 1)
            c = t & (TG - 1)
            jh0 = t * (n // 2)

            def at(ju, pos, extra=True):
                if ju % n != pos:
                    return False
                return c == ju // n if extra is True else jnp.logical_and(c == ju // n, extra)

            more = g < NP - 1
            gn = jnp.minimum(g + 1, NP - 1)
            q = (q_c[0], q_c[1])
            for pos in range(n):
                j = t * n + pos
                ro = (pos + 1) % 2
                r, jh, jhn = pos % 2, jh0 + pos // 2, jh0 + (pos + 1) // 2
                sk = sv = pos % R
                dk = pos + R - DL
                when(True if dk < n else t < T - 1, lambda: k_copy(jh0, dk).start())
                when(True if dk < n else t < T - 1, lambda: v_copy(jh0, dk).start())
                when(j + 1 + XL < UG, lambda: x_copy(jh0, pos + 1 + XL).start())
                when(at(10, pos, more), lambda: wq_copy(0, gn).start())
                when(at(14, pos, more), lambda: wq_copy(1, gn).start())
                when(at(18, pos, more), lambda: wo_copy(0, gn).start())
                when(at(22, pos, more), lambda: wo_copy(1, gn).start())
                o, s, new = {}, {}, {}
                for st in seq:
                    if st in 'abmzt':
                        if not o:
                            v_copy(jh0, pos).wait()
                        o[st] = pv_part(st, sv, new.get(0, (None,))[0], new.get(1, (None,))[0])
                        if len(o) == 5:
                            oj = pv_join(o, new[0][1], new[1][1])
                    elif st in 'AB':
                        if not s:
                            k_copy(jh0, pos).wait()
                        h = 'AB'.index(st)
                        s[h] = _nn(q[h], k_buf[sk, 128 * h:128 * h + 256, :])
                        if 'XY'[h] not in seq:
                            new[h] = softmax(s[h])
                    elif st in 'XY':
                        h = 'XY'.index(st)
                        new[h] = softmax(s[h])
                    elif st == 'Q':
                        when(at(UG - 1, pos, more), lambda: wq_copy(0, gn).wait())
                        when(at(0, pos), lambda: wq_copy(1, g).wait())
                        when(j + 1 < UG, lambda: x_copy(jh0, pos + 1).wait())
                        qn = Q(ro, jhn)
                    elif st == 'O':
                        when(at(0, pos), lambda: wo_copy(0, g).wait())
                        when(at(1, pos), lambda: wo_copy(1, g).wait())
                        O(r, jh, oj)
                        when(g == NP - 1, lambda: out_copy(r, jh & (B - 1)).start())
                q = qn
            q_c[0], q_c[1] = q
            return carry

        lax.fori_loop(0, T, body, 0)

        pltpu.make_async_copy(o_buf, o_buf, o_sem).wait()

    @jax.jit
    def fn(A_x, A_k_cache, A_v_cache, A_wq, A_wo, B_x, B_k_cache, B_v_cache, B_wq, B_wo):
        tr = lambda a: jnp.swapaxes(a, 2, 3).reshape(B, H * DH, SK)
        return pl.pallas_call(
            kernel,
            in_specs=[pl.BlockSpec(memory_space=pl.ANY)] * 10,
            out_specs=pl.BlockSpec(memory_space=pl.ANY),
            out_shape=jax.ShapeDtypeStruct((B, SQ, 2 * D), A_x.dtype),
            scratch_shapes=[
                pltpu.VMEM((2, B, SQ, D), bf16),
                pltpu.VMEM((2, NP, D, PW), bf16),
                pltpu.VMEM((2, NP, PW, D), bf16),
                pltpu.VMEM((R, PW, SK), bf16),
                pltpu.VMEM((R, PW, SK), bf16),
                pltpu.VMEM((2, B, SQ, D), f32),
                pltpu.VMEM((2, B, SQ, D), A_x.dtype),
                pltpu.VMEM((2, SQ, 256), bf16),
                pltpu.SemaphoreType.DMA((2 * R + 4 + 2 * B,)),
                pltpu.SemaphoreType.DMA,
            ],
            compiler_params=pltpu.CompilerParams(vmem_limit_bytes=vmem_mb * 1024 * 1024, flags=flags, disable_bounds_checks=True),
            name="attn",
        )(A_x, tr(A_k_cache), tr(A_v_cache), A_wq, A_wo, B_x, tr(B_k_cache), tr(B_v_cache), B_wq, B_wo)
    return fn


_fn = make(n=16, seq='ABzatbmQO')


@jax.jit
def pallas_concat_heads__gqa_block_cached__mha_block_cached__near_ridge_kernel(
    A_x, A_k_cache, A_v_cache, A_wq, A_wo, B_x, B_k_cache, B_v_cache, B_wq, B_wo
):
    return _fn(A_x, A_k_cache, A_v_cache, A_wq, A_wo, B_x, B_k_cache, B_v_cache, B_wq, B_wo)
```

```python
import jax
import jax.numpy as jnp
import numpy as np
from jax import lax
import jax.experimental.pallas as pl
import jax.experimental.pallas.tpu as pltpu

B, SQ, D = 16, 160, 640
H, SK, DH = 32, 512, 192
PW = 2 * DH
NP = H // 2
UG = 2 * B
NU = NP * UG
QM = 128
QL = SQ - QM
QSCALE = float(DH ** -0.5 * np.log2(np.e))

NN = (((1,), (0,)), ((), ()))
NT = (((1,), (1,)), ((), ()))
f32, bf16 = jnp.float32, jnp.bfloat16


def _nn(a, b):
    return lax.dot_general(a, b, NN, preferred_element_type=f32)


def _nt(a, b):
    return lax.dot_general(a, b, NT, preferred_element_type=f32)


def make(n=8, R=8, seq='ABdzatbmQO', vmem_mb=110, flags=None, XL=6, DL=1, run=None, s0=None, s1=None, sl=None, sm=0, qs_=0):
    flags = dict(flags or {}, XLA_TPU_RESCHEDULE_DMA_DONES=True)
    T = NU // n
    TG = UG // n
    R = min(R, n)
    run = run or n // 2
    assert n % R == 0 and n % (2 * run) == 0
    seqs = [seq] * n
    seqs[0], seqs[1], seqs[-1] = s0 or seq, s1 or seq, sl or seq

    def kernel(ax, ak, av, awq, awo, bx, bk, bv, bwq, bwo, out_hbm,
               x_buf, wq_buf, wo_buf, k_buf, v_buf, acc, o_buf, q_c, sems, o_sem):
        x_hbm, k_hbm, v_hbm = (ax, bx), (ak, bk), (av, bv)
        wq_hbm, wo_hbm = (awq, bwq), (awo, bwo)
        lo = lax.broadcasted_iota(jnp.int32, (SQ, 128), 1) < 64
        lo_m = lax.broadcasted_iota(jnp.int32, (QM, 128), 1) < 64
        lo_l = lax.broadcasted_iota(jnp.int32, (QL, 128), 1) < 64

        def al(i, m):
            return i if isinstance(i, int) else pl.multiple_of(i, m)

        def unit(t, d):
            jh = t * (n // 2) + d // (2 * run) * run + d % run
            return d // run % 2, (jh >> 4) & (NP - 1), jh & (B - 1)

        def when(cond, f):
            if isinstance(cond, bool):
                if cond:
                    f()
            else:
                pl.when(cond)(f)

        def k_copy(t, d):
            r, g, b = unit(t, d)
            return pltpu.make_async_copy(k_hbm[r].at[b, pl.ds(al(g * PW, PW), PW), :], k_buf.at[d % R], sems.at[d % R])

        def v_copy(t, d):
            r, g, b = unit(t, d)
            return pltpu.make_async_copy(v_hbm[r].at[b, pl.ds(al(g * PW, PW), PW), :], v_buf.at[d % R], sems.at[R + d % R])

        def x_copy(t, d):
            r, _, b = unit(t, d)
            return pltpu.make_async_copy(x_hbm[r].at[b], x_buf.at[r, b], sems.at[2 * R + 4 + r * B + b])

        def wq_copy(r, g):
            return pltpu.make_async_copy(wq_hbm[r].at[:, pl.ds(al(g * PW, 128), PW)], wq_buf.at[r, g], sems.at[2 * R + r])

        def wo_copy(r, g):
            return pltpu.make_async_copy(wo_hbm[r].at[pl.ds(al(g * PW, PW), PW), :], wo_buf.at[r, g], sems.at[2 * R + 2 + r])

        def out_copy(r, b):
            return pltpu.make_async_copy(o_buf.at[r, b], out_hbm.at[b, :, pl.ds(r * D, D)], o_sem)

        def q_split(q0, q1, q2):
            qa = jnp.concatenate([q0, jnp.where(lo, q1, 0.0)], axis=1).astype(bf16)
            qb = jnp.concatenate([jnp.where(lo, 0.0, q1), q2], axis=1).astype(bf16)
            return qa, qb

        def Q(r, g, b):
            if qs_ == 1:
                q = _nn(x_buf[r, b, :, 0:512], wq_buf[r, g, 0:512, :])
                w = wq_buf[r, g, 512:640, 0:256]
                e = jnp.concatenate([_nn(x_buf[r, b, 0:80, 512:640], w), _nn(x_buf[r, b, 80:160, 512:640], w)], axis=0)
                e = jnp.concatenate([e, _nn(x_buf[r, b, :, 512:640], wq_buf[r, g, 512:640, 256:384])], axis=1)
                q = (q + e) * QSCALE
            elif qs_ == 2:
                w = wq_buf[r, g, 384:640, 0:128]
                e = jnp.concatenate([_nn(x_buf[r, b, 0:80, 384:640], w), _nn(x_buf[r, b, 80:160, 384:640], w)], axis=0)
                q0 = e + _nn(x_buf[r, b, :, 0:384], wq_buf[r, g, 0:384, 0:128])
                q = jnp.concatenate([q0, _nn(x_buf[r, b], wq_buf[r, g, :, 128:384])], axis=1) * QSCALE
            else:
                q = _nn(x_buf[r, b], wq_buf[r, g]) * QSCALE
            return q_split(q[:, 0:128], q[:, 128:256], q[:, 256:384])

        def softmax(s):
            m = jnp.max(s, axis=-1, keepdims=True)
            p = jnp.exp2(s - m)
            l = jnp.sum(p, axis=-1, keepdims=True)
            if sm & 2:
                rl = 1.0 / l
            else:
                rl = pl.reciprocal(l, approx=True)
                rl = rl * (2.0 - l * rl)
            if sm & 1:
                pb = p.astype(bf16)
                return (pb, pb[:QM], pb[QM:]), rl
            return (p.astype(bf16), p[:QM].astype(bf16), p[QM:].astype(bf16)), rl

        def pv_part(k, slot, pa, pb):
            if k == 'z':
                return _nt(pa[0], v_buf[slot, 0:128, :])
            if k == 't':
                return _nt(pb[0], v_buf[slot, 256:384, :])
            if k == 'a':
                return _nt(v_buf[slot, 128:192, :], pa[1])
            if k == 'b':
                return _nt(v_buf[slot, 192:256, :], pb[1])
            return _nt(jnp.concatenate([pa[2], pb[2]], axis=0), v_buf[slot, 128:256, :])

        def pv_join(o, ra, rb):
            om = jnp.concatenate([o['a'], o['b']], axis=0).T * jnp.where(lo_m, ra[:QM], rb[:QM])
            ol = jnp.where(lo_l, o['m'][:QL] * ra[QM:], o['m'][QL:] * rb[QM:])
            return jnp.concatenate([o['z'] * ra, jnp.concatenate([om, ol], axis=0), o['t'] * rb], axis=1).astype(bf16)

        def O(r, g, b, o):
            tot = jnp.where(g == 0, 0.0, acc[r, b]) + _nn(o, wo_buf[r, g])
            acc[r, b] = tot
            o_buf[r, b] = tot.astype(o_buf.dtype)

        wq_copy(0, 0).start()
        x_copy(0, 0).start()
        for j in range(max(R, XL, run + 1)):
            if j < R - DL:
                k_copy(0, j).start()
                v_copy(0, j).start()
            if j == run - 1:
                wq_copy(1, 0).start()
            if j < XL:
                x_copy(0, j + 1).start()
            if j in (0, run):
                wo_copy(j // run, 0).start()
        wq_copy(0, 0).wait()
        x_copy(0, 0).wait()
        q_c[0], q_c[1] = Q(0, 0, 0)

        def body(t, carry):
            g = t >> (TG.bit_length() - 1)
            c = t & (TG - 1)

            def at(ju, pos, extra=True):
                if ju % n != pos:
                    return False
                return c == ju // n if extra is True else jnp.logical_and(c == ju // n, extra)

            more = g < NP - 1
            gn = jnp.minimum(g + 1, NP - 1)
            q = (q_c[0], q_c[1])
            for pos in range(n):
                j = t * n + pos
                slot = pos % R
                o, s, qs = {}, {}, {}
                for st in seqs[pos]:
                    if st == 'd':
                        dk = pos + R - DL
                        when(True if dk < n else t < T - 1, lambda: k_copy(t, dk).start())
                        when(True if dk < n else t < T - 1, lambda: v_copy(t, dk).start())
                        when(j + 1 + XL < UG, lambda: x_copy(t, pos + 1 + XL).start())
                        when(at(18, pos, more), lambda: wq_copy(0, gn).start())
                        when(at(21, pos, more), lambda: wo_copy(0, gn).start())
                        when(at(24, pos, more), lambda: wq_copy(1, gn).start())
                        when(at(27, pos, more), lambda: wo_copy(1, gn).start())
                    elif st in 'abmzt':
                        if not o:
                            v_copy(t, pos).wait()
                        o[st] = pv_part(st, slot, s.get(0, (None,))[0], s.get(1, (None,))[0])
                    elif st in 'AB':
                        if not s:
                            k_copy(t, pos).wait()
                        h = 'AB'.index(st)
                        s[h] = softmax(_nn(q[h], k_buf[slot, 128 * h:128 * h + 256, :]))
                    elif st in 'Q012':
                        if not qs:
                            when(at(UG - 1, pos, more), lambda: wq_copy(0, gn).wait())
                            when(at(run - 1, pos), lambda: wq_copy(1, g).wait())
                            when(j + 1 < UG, lambda: x_copy(t, pos + 1).wait())
                        if st == 'Q':
                            qn = Q(*unit(t, pos + 1))
                        else:
                            rn, gq, bn = unit(t, pos + 1)
                            i = int(st)
                            qs[i] = _nn(x_buf[rn, bn], wq_buf[rn, gq, :, 128 * i:128 * i + 128]) * QSCALE
                            if len(qs) == 3:
                                qn = q_split(qs[0], qs[1], qs[2])
                    elif st == 'O':
                        when(at(0, pos), lambda: wo_copy(0, g).wait())
                        when(at(run, pos), lambda: wo_copy(1, g).wait())
                        r, go, b = unit(t, pos)
                        O(r, go, b, pv_join(o, s[0][1], s[1][1]))
                        when(g == NP - 1, lambda: out_copy(r, b).start())
                q = qn
            q_c[0], q_c[1] = q
            return carry

        lax.fori_loop(0, T, body, 0)
        pltpu.make_async_copy(o_buf, o_buf, o_sem).wait()

    @jax.jit
    def fn(A_x, A_k_cache, A_v_cache, A_wq, A_wo, B_x, B_k_cache, B_v_cache, B_wq, B_wo):
        tr = lambda a: jnp.swapaxes(a, 2, 3).reshape(B, H * DH, SK)
        return pl.pallas_call(
            kernel,
            in_specs=[pl.BlockSpec(memory_space=pl.ANY)] * 10,
            out_specs=pl.BlockSpec(memory_space=pl.ANY),
            out_shape=jax.ShapeDtypeStruct((B, SQ, 2 * D), A_x.dtype),
            scratch_shapes=[
                pltpu.VMEM((2, B, SQ, D), bf16),
                pltpu.VMEM((2, NP, D, PW), bf16),
                pltpu.VMEM((2, NP, PW, D), bf16),
                pltpu.VMEM((R, PW, SK), bf16),
                pltpu.VMEM((R, PW, SK), bf16),
                pltpu.VMEM((2, B, SQ, D), f32),
                pltpu.VMEM((2, B, SQ, D), A_x.dtype),
                pltpu.VMEM((2, SQ, 256), bf16),
                pltpu.SemaphoreType.DMA((2 * R + 4 + 2 * B,)),
                pltpu.SemaphoreType.DMA,
            ],
            compiler_params=pltpu.CompilerParams(vmem_limit_bytes=vmem_mb * 1024 * 1024, flags=flags, disable_bounds_checks=True),
            name="attn",
        )(A_x, tr(A_k_cache), tr(A_v_cache), A_wq, A_wo, B_x, tr(B_k_cache), tr(B_v_cache), B_wq, B_wo)
    return fn


_fn = make(n=16, seq='ABzatbmQdO', qs_=1)


@jax.jit
def pallas_concat_heads__gqa_block_cached__mha_block_cached__near_ridge_kernel(
    A_x, A_k_cache, A_v_cache, A_wq, A_wo, B_x, B_k_cache, B_v_cache, B_wq, B_wo
):
    return _fn(A_x, A_k_cache, A_v_cache, A_wq, A_wo, B_x, B_k_cache, B_v_cache, B_wq, B_wo)
```

```python
import jax
import jax.numpy as jnp
import numpy as np
from jax import lax
import jax.experimental.pallas as pl
import jax.experimental.pallas.tpu as pltpu

B, SQ, D = 16, 160, 640
H, SK, DH = 32, 512, 192
PW = 2 * DH
NP = H // 2
QM = 128
QL = SQ - QM
QSCALE = float(DH ** -0.5 * np.log2(np.e))

RUN = 8
N = 2 * RUN
TG = B // RUN
T = NP * TG

f32, bf16 = jnp.float32, jnp.bfloat16


def _nn(a, b):
    return lax.dot_general(a, b, (((1,), (0,)), ((), ())), preferred_element_type=f32)


def _nt(a, b):
    return lax.dot_general(a, b, (((1,), (1,)), ((), ())), preferred_element_type=f32)


def _low_half(rows):
    return lax.broadcasted_iota(jnp.int32, (rows, 128), 1) < 64


def _aligned(i, m):
    return i if isinstance(i, int) else pl.multiple_of(i, m)


def _softmax(s):
    p = jnp.exp2(s - jnp.max(s, axis=-1, keepdims=True))
    l = jnp.sum(p, axis=-1, keepdims=True)
    r = pl.reciprocal(l, approx=True)
    r = r * (2.0 - l * r)
    return p.astype(bf16), p[:QM].astype(bf16), p[QM:].astype(bf16), r


def make(R=8, G=2, T0=2, XL=6, W=(2, 5, 8, 11), dpos=0):
    def kernel(ax, ak, av, awq, awo, bx, bk, bv, bwq, bwo, out_hbm,
               x_buf, wq_buf, wo_buf, k_buf, v_buf, acc, o_buf, q_next, sems, o_sem):
        x_hbm, k_hbm, v_hbm = (ax, bx), (ak, bk), (av, bv)
        wq_hbm, wo_hbm = (awq, bwq), (awo, bwo)

        def kv_copy(hbm, buf, sem0, unit, slot, m):
            r, g, b = unit
            return pltpu.make_async_copy(
                hbm[r].at[pl.ds(b, m), pl.ds(_aligned(g * PW, PW), PW), :],
                buf.at[pl.ds(slot, m)], sems.at[sem0 + slot])

        def k_copy(unit, slot, m=1):
            return kv_copy(k_hbm, k_buf, 0, unit, slot, m)

        def v_copy(unit, slot, m=1):
            return kv_copy(v_hbm, v_buf, R, unit, slot, m)

        def wq_copy(r, g):
            return pltpu.make_async_copy(
                wq_hbm[r].at[:, pl.ds(_aligned(g * PW, 128), PW)], wq_buf.at[r, g], sems.at[2 * R + r])

        def wo_copy(r, g):
            return pltpu.make_async_copy(
                wo_hbm[r].at[pl.ds(_aligned(g * PW, PW), PW), :], wo_buf.at[r, g], sems.at[2 * R + 2 + r])

        def x_copy(unit):
            r, _, b = unit
            return pltpu.make_async_copy(x_hbm[r].at[b], x_buf.at[r, b], sems.at[2 * R + 4 + r * B + b])

        def out_copy(unit):
            r, _, b = unit
            return pltpu.make_async_copy(o_buf.at[r, b], out_hbm.at[b, :, pl.ds(r * D, D)], o_sem)

        def project_q(unit):
            r, g, b = unit
            w = wq_buf[r, g, 512:D, 0:256]
            e = jnp.concatenate(
                [_nn(x_buf[r, b, 0:SQ // 2, 512:D], w), _nn(x_buf[r, b, SQ // 2:SQ, 512:D], w)], axis=0)
            e = jnp.concatenate([e, _nn(x_buf[r, b, :, 512:D], wq_buf[r, g, 512:D, 256:PW])], axis=1)
            q = (_nn(x_buf[r, b, :, 0:512], wq_buf[r, g, 0:512, :]) + e) * QSCALE
            lo = _low_half(SQ)
            qa = jnp.concatenate([q[:, 0:128], jnp.where(lo, q[:, 128:256], 0.0)], axis=1)
            qb = jnp.concatenate([jnp.where(lo, 0.0, q[:, 128:256]), q[:, 256:PW]], axis=1)
            return qa.astype(bf16), qb.astype(bf16)

        def weigh_values(slot, sa, sb):
            pa, pa_m, pa_l, ra = sa
            pb, pb_m, pb_l, rb = sb
            o0 = _nt(pa, v_buf[slot, 0:128, :])
            o1a = _nt(v_buf[slot, 128:DH, :], pa_m)
            o2 = _nt(pb, v_buf[slot, 256:PW, :])
            o1b = _nt(v_buf[slot, DH:256, :], pb_m)
            o1l = _nt(jnp.concatenate([pa_l, pb_l], axis=0), v_buf[slot, 128:256, :])
            o1m = jnp.concatenate([o1a, o1b], axis=0).T * jnp.where(_low_half(QM), ra[:QM], rb[:QM])
            o1l = jnp.where(_low_half(QL), o1l[:QL] * ra[QM:], o1l[QL:] * rb[QM:])
            o1 = jnp.concatenate([o1m, o1l], axis=0)
            return jnp.concatenate([o0 * ra, o1, o2 * rb], axis=1).astype(bf16)

        def project_out(unit, o):
            r, g, b = unit
            total = jnp.where(g == 0, 0.0, acc[r, b]) + _nn(o, wo_buf[r, g])
            acc[r, b] = total
            o_buf[r, b] = total.astype(o_buf.dtype)

        first = lambda d: (d // RUN % 2, 0, d // N * RUN + d % RUN)
        wq_copy(0, 0).start()
        x_copy(first(0)).start()
        for d in range(max(R - G, XL, RUN + 1)):
            if d < R - G:
                k_copy(first(d), d).start()
                v_copy(first(d), d).start()
            if d == RUN - 1:
                wq_copy(1, 0).start()
            if d < XL:
                x_copy(first(d + 1)).start()
            if d in (0, RUN):
                wo_copy(d // RUN, 0).start()
        wq_copy(0, 0).wait()
        x_copy(first(0)).wait()
        q_next[0], q_next[1] = project_q(first(0))

        def step(t, carry):
            g, c = lax.div(t, TG), lax.rem(t, TG)
            t1 = lax.rem(t + 1, T)
            g1, c1 = lax.div(t1, TG), lax.rem(t1, TG)
            gn = jnp.minimum(g + 1, NP - 1)
            pair_begins = c == 0
            pair_ends = jnp.logical_and(c == TG - 1, g < NP - 1)

            def unit(d):
                if d < N:
                    return d // RUN, g, c * RUN + d % RUN
                return (d - N) // RUN, g1, c1 * RUN + d % RUN

            def kv_start(copy, d):
                td = t + d // N
                pl.when(td < T0)(lambda: copy(unit(d), d % R).start())
                if d % G == 0:
                    pl.when(jnp.logical_and(td >= T0, td < T))(lambda: copy(unit(d), d % R, G).start())

            def kv_wait(copy, d):
                pl.when(t < T0)(lambda: copy(unit(d), d % R).wait())
                if d % G == 0:
                    pl.when(t >= T0)(lambda: copy(unit(d), d % R, G).wait())

            def prefetch(d):
                kv_start(k_copy, d + R - G)
                kv_start(v_copy, d + R - G)
                pl.when(t + (d + 1 + XL) // N < TG)(lambda: x_copy(unit(d + 1 + XL)).start())
                weights = dict(zip(W, ((wq_copy, 0), (wo_copy, 0), (wq_copy, 1), (wo_copy, 1))))
                if d in weights:
                    pl.when(pair_ends)(lambda: weights[d][0](weights[d][1], gn).start())

            qa, qb = q_next[0], q_next[1]
            for d in range(N):
                slot = d % R
                kv_wait(k_copy, d)
                sa = _softmax(_nn(qa, k_buf[slot, 0:256, :]))
                sb = _softmax(_nn(qb, k_buf[slot, 128:PW, :]))
                if dpos == 1:
                    prefetch(d)
                kv_wait(v_copy, d)
                o = weigh_values(slot, sa, sb)
                if dpos == 2:
                    prefetch(d)

                if d + 1 == RUN:
                    pl.when(pair_begins)(lambda: wq_copy(1, g).wait())
                if d + 1 == N:
                    pl.when(pair_ends)(lambda: wq_copy(0, gn).wait())
                pl.when(t + (d + 1) // N < TG)(lambda: x_copy(unit(d + 1)).wait())
                qa, qb = project_q(unit(d + 1))
                if dpos == 0:
                    prefetch(d)

                if d % RUN == 0:
                    pl.when(pair_begins)(lambda: wo_copy(d // RUN, g).wait())
                project_out(unit(d), o)
                pl.when(g == NP - 1)(lambda: out_copy(unit(d)).start())
            q_next[0], q_next[1] = qa, qb
            return carry

        lax.fori_loop(0, T, step, 0)
        pltpu.make_async_copy(out_hbm, out_hbm, o_sem).wait()

    @jax.jit
    def fn(A_x, A_k_cache, A_v_cache, A_wq, A_wo, B_x, B_k_cache, B_v_cache, B_wq, B_wo):
        transposed = lambda a: jnp.swapaxes(a, 2, 3).reshape(B, H * DH, SK)
        return pl.pallas_call(
            kernel,
            in_specs=[pl.BlockSpec(memory_space=pl.ANY)] * 10,
            out_specs=pl.BlockSpec(memory_space=pl.ANY),
            out_shape=jax.ShapeDtypeStruct((B, SQ, 2 * D), A_x.dtype),
            scratch_shapes=[
                pltpu.VMEM((2, B, SQ, D), bf16),
                pltpu.VMEM((2, NP, D, PW), bf16),
                pltpu.VMEM((2, NP, PW, D), bf16),
                pltpu.VMEM((R, PW, SK), bf16),
                pltpu.VMEM((R, PW, SK), bf16),
                pltpu.VMEM((2, B, SQ, D), f32),
                pltpu.VMEM((2, B, SQ, D), A_x.dtype),
                pltpu.VMEM((2, SQ, 256), bf16),
                pltpu.SemaphoreType.DMA((2 * R + 4 + 2 * B,)),
                pltpu.SemaphoreType.DMA,
            ],
            compiler_params=pltpu.CompilerParams(
                vmem_limit_bytes=100 * 1024 * 1024,
                disable_bounds_checks=True,
                flags={"XLA_TPU_RESCHEDULE_DMA_DONES": True},
            ),
            name="attn",
        )(A_x, transposed(A_k_cache), transposed(A_v_cache), A_wq, A_wo,
          B_x, transposed(B_k_cache), transposed(B_v_cache), B_wq, B_wo)
    return fn


_fn = make()


@jax.jit
def pallas_concat_heads__gqa_block_cached__mha_block_cached__near_ridge_kernel(
    A_x, A_k_cache, A_v_cache, A_wq, A_wo, B_x, B_k_cache, B_v_cache, B_wq, B_wo
):
    return _fn(A_x, A_k_cache, A_v_cache, A_wq, A_wo, B_x, B_k_cache, B_v_cache, B_wq, B_wo)
```

```python
import jax
import jax.numpy as jnp
import numpy as np
from jax import lax
import jax.experimental.pallas as pl
import jax.experimental.pallas.tpu as pltpu

B, SQ, D = 16, 160, 640
H, SK, DH = 32, 512, 192
PW = 2 * DH
NP = H // 2
QM = 128
QL = SQ - QM
QSCALE = float(DH ** -0.5 * np.log2(np.e))

RUN = 8
N = 2 * RUN
TG = B // RUN
T = NP * TG
R = 8

f32, bf16 = jnp.float32, jnp.bfloat16
_reciprocal = pltpu.reciprocal if hasattr(pltpu, "reciprocal") else pl.reciprocal


def _nn(a, b):
    return lax.dot_general(a, b, (((1,), (0,)), ((), ())), preferred_element_type=f32)


def _nt(a, b):
    return lax.dot_general(a, b, (((1,), (1,)), ((), ())), preferred_element_type=f32)


def _low_half(rows):
    return lax.broadcasted_iota(jnp.int32, (rows, 128), 1) < 64


def _aligned(i, m):
    return i if isinstance(i, int) else pl.multiple_of(i, m)


def _softmax(s):
    p = jnp.exp2(s - jnp.max(s, axis=-1, keepdims=True))
    l = jnp.sum(p, axis=-1, keepdims=True)
    r = _reciprocal(l, approx=True)
    r = r * (2.0 - l * r)
    return p.astype(bf16), p[:QM].astype(bf16), p[QM:].astype(bf16), r


def _kernel(ax, ak, av, awq, awo, bx, bk, bv, bwq, bwo, out_hbm,
            x_buf, wq_buf, wo_buf, k_buf, v_buf, acc, o_buf, q_next, in_sems, out_sem):
    x_hbm, k_hbm, v_hbm = (ax, bx), (ak, bk), (av, bv)
    wq_hbm, wo_hbm = (awq, bwq), (awo, bwo)

    def k_copy(unit, slot):
        r, g, b = unit
        return pltpu.make_async_copy(
            k_hbm[r].at[b, pl.ds(_aligned(g * PW, PW), PW), :], k_buf.at[slot], in_sems.at[slot])

    def v_copy(unit, slot):
        r, g, b = unit
        return pltpu.make_async_copy(
            v_hbm[r].at[b, pl.ds(_aligned(g * PW, PW), PW), :], v_buf.at[slot], in_sems.at[R + slot])

    def wq_copy(r, g):
        return pltpu.make_async_copy(
            wq_hbm[r].at[:, pl.ds(_aligned(g * PW, 128), PW)], wq_buf.at[r, g], in_sems.at[2 * R + r])

    def wo_copy(r, g):
        return pltpu.make_async_copy(
            wo_hbm[r].at[pl.ds(_aligned(g * PW, PW), PW), :], wo_buf.at[r, g], in_sems.at[2 * R + 2 + r])

    def x_copy(unit):
        r, _, b = unit
        return pltpu.make_async_copy(x_hbm[r].at[b], x_buf.at[r, b], in_sems.at[2 * R + 4 + r * B + b])

    def out_copy(unit):
        r, _, b = unit
        return pltpu.make_async_copy(o_buf.at[r, b], out_hbm.at[b, :, pl.ds(r * D, D)], out_sem)

    def project_q(unit):
        r, g, b = unit
        w = wq_buf[r, g, 512:D, 0:256]
        e = jnp.concatenate(
            [_nn(x_buf[r, b, 0:SQ // 2, 512:D], w), _nn(x_buf[r, b, SQ // 2:SQ, 512:D], w)], axis=0)
        e = jnp.concatenate([e, _nn(x_buf[r, b, :, 512:D], wq_buf[r, g, 512:D, 256:PW])], axis=1)
        q = (_nn(x_buf[r, b, :, 0:512], wq_buf[r, g, 0:512, :]) + e) * QSCALE
        lo = _low_half(SQ)
        qa = jnp.concatenate([q[:, 0:128], jnp.where(lo, q[:, 128:256], 0.0)], axis=1)
        qb = jnp.concatenate([jnp.where(lo, 0.0, q[:, 128:256]), q[:, 256:PW]], axis=1)
        return qa.astype(bf16), qb.astype(bf16)

    def weigh_values(slot, sa, sb):
        pa, pa_main, pa_left, ra = sa
        pb, pb_main, pb_left, rb = sb
        o0 = _nt(pa, v_buf[slot, 0:128, :])
        o1a = _nt(v_buf[slot, 128:DH, :], pa_main)
        o2 = _nt(pb, v_buf[slot, 256:PW, :])
        o1b = _nt(v_buf[slot, DH:256, :], pb_main)
        o1l = _nt(jnp.concatenate([pa_left, pb_left], axis=0), v_buf[slot, 128:256, :])
        o1m = jnp.concatenate([o1a, o1b], axis=0).T * jnp.where(_low_half(QM), ra[:QM], rb[:QM])
        o1l = jnp.where(_low_half(QL), o1l[:QL] * ra[QM:], o1l[QL:] * rb[QM:])
        o1 = jnp.concatenate([o1m, o1l], axis=0)
        return jnp.concatenate([o0 * ra, o1, o2 * rb], axis=1).astype(bf16)

    def project_out(unit, o):
        r, g, b = unit
        total = jnp.where(g == 0, 0.0, acc[r, b]) + _nn(o, wo_buf[r, g])
        acc[r, b] = total
        o_buf[r, b] = total.astype(o_buf.dtype)

    def first(d):
        return d // RUN, 0, d % RUN

    wq_copy(0, 0).start()
    x_copy(first(0)).start()
    for d in range(RUN + 1):
        if d < R - 1:
            k_copy(first(d), d).start()
            v_copy(first(d), d).start()
            x_copy(first(d + 1)).start()
        if d + 1 == RUN:
            wq_copy(1, 0).start()
        if d % RUN == 0:
            wo_copy(d // RUN, 0).start()
    wq_copy(0, 0).wait()
    x_copy(first(0)).wait()
    q_next[0], q_next[1] = project_q(first(0))

    def step(t, carry):
        g, c = lax.div(t, TG), lax.rem(t, TG)
        t1 = lax.rem(t + 1, T)
        g1, c1 = lax.div(t1, TG), lax.rem(t1, TG)
        g_next = jnp.minimum(g + 1, NP - 1)
        pair_begins = c == 0
        next_pair_follows = jnp.logical_and(c == TG - 1, g < NP - 1)
        weight_prefetch = {2: (wq_copy, 0), 5: (wo_copy, 0), 8: (wq_copy, 1), 11: (wo_copy, 1)}

        def unit(d):
            if d < N:
                return d // RUN, g, c * RUN + d % RUN
            return (d - N) // RUN, g1, c1 * RUN + d % RUN

        def prefetch(d):
            e = d + R - 1
            for copy in (k_copy, v_copy):
                if e < N:
                    copy(unit(e), e % R).start()
                else:
                    pl.when(t < T - 1)(lambda: copy(unit(e), e % R).start())
            pl.when(t + (d + R) // N < TG)(lambda: x_copy(unit(d + R)).start())
            if d in weight_prefetch:
                w_copy, r = weight_prefetch[d]
                pl.when(next_pair_follows)(lambda: w_copy(r, g_next).start())

        qa, qb = q_next[0], q_next[1]
        for d in range(N):
            slot = d % R
            k_copy(unit(d), slot).wait()
            sa = _softmax(_nn(qa, k_buf[slot, 0:256, :]))
            sb = _softmax(_nn(qb, k_buf[slot, 128:PW, :]))
            v_copy(unit(d), slot).wait()
            o = weigh_values(slot, sa, sb)

            if d + 1 == RUN:
                pl.when(pair_begins)(lambda: wq_copy(1, g).wait())
            if d + 1 == N:
                pl.when(next_pair_follows)(lambda: wq_copy(0, g_next).wait())
            pl.when(t + (d + 1) // N < TG)(lambda: x_copy(unit(d + 1)).wait())
            qa, qb = project_q(unit(d + 1))
            prefetch(d)

            if d % RUN == 0:
                pl.when(pair_begins)(lambda: wo_copy(d // RUN, g).wait())
            project_out(unit(d), o)
            pl.when(g == NP - 1)(lambda: out_copy(unit(d)).start())
        q_next[0], q_next[1] = qa, qb
        return carry

    lax.fori_loop(0, T, step, 0)
    pltpu.make_async_copy(out_hbm, out_hbm, out_sem).wait()


@jax.jit
def pallas_concat_heads__gqa_block_cached__mha_block_cached__near_ridge_kernel(
    A_x: jax.Array,
    A_k_cache: jax.Array,
    A_v_cache: jax.Array,
    A_wq: jax.Array,
    A_wo: jax.Array,
    B_x: jax.Array,
    B_k_cache: jax.Array,
    B_v_cache: jax.Array,
    B_wq: jax.Array,
    B_wo: jax.Array,
):
    def transposed(cache):
        return jnp.swapaxes(cache, 2, 3).reshape(B, H * DH, SK)

    return pl.pallas_call(
        _kernel,
        in_specs=[pl.BlockSpec(memory_space=pl.ANY)] * 10,
        out_specs=pl.BlockSpec(memory_space=pl.ANY),
        out_shape=jax.ShapeDtypeStruct((B, SQ, 2 * D), A_x.dtype),
        scratch_shapes=[
            pltpu.VMEM((2, B, SQ, D), bf16),
            pltpu.VMEM((2, NP, D, PW), bf16),
            pltpu.VMEM((2, NP, PW, D), bf16),
            pltpu.VMEM((R, PW, SK), bf16),
            pltpu.VMEM((R, PW, SK), bf16),
            pltpu.VMEM((2, B, SQ, D), f32),
            pltpu.VMEM((2, B, SQ, D), A_x.dtype),
            pltpu.VMEM((2, SQ, 256), bf16),
            pltpu.SemaphoreType.DMA((2 * R + 4 + 2 * B,)),
            pltpu.SemaphoreType.DMA,
        ],
        compiler_params=pltpu.CompilerParams(
            vmem_limit_bytes=100 * 1024 * 1024,
            disable_bounds_checks=True,
            flags={"XLA_TPU_RESCHEDULE_DMA_DONES": True},
        ),
        name="attn",
    )(A_x, transposed(A_k_cache), transposed(A_v_cache), A_wq, A_wo,
      B_x, transposed(B_k_cache), transposed(B_v_cache), B_wq, B_wo)
```
